```python
import os as _os
_os.environ.setdefault("JAX_PLATFORMS", "cpu")
import jax
import jax.numpy as jnp

def _softmax(x, axis=-1):
    return jax.nn.softmax(x, axis=axis)
def _gelu(x):
    return jax.nn.gelu(x, approximate=True)
def _silu(x):
    return jax.nn.silu(x)
def _sigmoid(x):
    return jax.nn.sigmoid(x)
def _layernorm(x, axis=-1, eps=1e-5):
    m = jnp.mean(x, axis=axis, keepdims=True)
    v = jnp.var(x, axis=axis, keepdims=True)
    return (x - m) / jnp.sqrt(v + eps)
def _scatter_add(tgt, idx, src, axis=0):
    return tgt.at[idx].add(src)
def _segment_sum(src, seg, n):
    return jax.ops.segment_sum(src, seg, n)
class _Rng:
    def __init__(self, key):
        self._k = key
    def _next(self):
        self._k, sub = jax.random.split(self._k)
        return sub
    def normal(self, shape):
        return jax.random.normal(self._next(), shape, dtype=jnp.bfloat16)
    def randint(self, lo, hi, shape):
        return jax.random.randint(self._next(), shape, lo, hi, dtype=jnp.int32)
    def uniform(self, shape, lo=0.0, hi=1.0):
        return jax.random.uniform(self._next(), shape, jnp.bfloat16, lo, hi)
    def permutation(self, n):
        return jax.random.permutation(self._next(), n)


kernel_name = 'standalone__mha_block_cached__near_ridge'

def setup_inputs():
    _rng = _Rng(jax.random.key(int.from_bytes(__import__("os").urandom(4), "little")))
    _w = (lambda a: (lambda t: t.astype(jnp.bfloat16) if jnp.issubdtype(t.dtype, jnp.floating) else t)(jnp.asarray(a)))
    B, Sq, D = 16, 64, 576
    H, Sk, Dh = 32, 64, 128
    return {
        "x": _w((lambda *s: _rng.normal(s) * 0.8)(B, Sq, D)),
        "k_cache": _w((lambda *s: _rng.normal(s) * 0.8)(B, H, Sk, Dh)),
        "v_cache": _w((lambda *s: _rng.normal(s) * 0.05)(B, H, Sk, Dh)),
        "wq": _w((lambda *s: _rng.normal(s) * 0.8)(D, H * Dh) * (D ** -0.5)),
        "wo": _w((lambda *s: _rng.normal(s) * 0.05)(H * Dh, D) * ((H * Dh) ** -0.5)),
    }

def reference(x, k_cache, v_cache, wq, wo):
    B, Sq, D = x.shape
    H, Dh = 32, 128
    q = (lambda x, *d: x.transpose(*d))((x @ wq).reshape(B, Sq, H, Dh), 0, 2, 1, 3)
    scores = jnp.einsum("bhqd,bhkd->bhqk", q, k_cache) * (Dh ** -0.5)
    p = _softmax(scores, axis=-1)
    o = jnp.einsum("bhqk,bhkd->bhqd", p, v_cache)
    return (lambda x, *d: x.transpose(*d))(o, 0, 2, 1, 3).reshape(B, Sq, H * Dh) @ wo
```

```python
import jax
import jax.numpy as jnp
import jax.experimental.pallas as pl
import jax.experimental.pallas.tpu as pltpu

B, SQ, D, H, SK, DH = 16, 64, 576, 32, 64, 128
R = B * SQ
G = 4
NG = H // G
GW = G * DH
LAG = 4
W = 4
XSPLIT = (0, 128, 384, 1024)
LOG2E = 1.4426950408889634
NT = (((1,), (1,)), ((), ()))

NX = len(XSPLIT) - 1
S_WQ1 = NX + 1
S_REG = S_WQ1 + 1
S_TAIL = S_REG + (NG - 2)
NS = S_TAIL + 1


def _body(x_hbm, k_hbm, v_hbm, wq_hbm, wot_hbm, o_hbm,
          x_v, k_v, v_v, wq_v, wot_v, acc_ref, q_ref, oh_ref, zs_ref, sems, osem):
    def cp(kind, g, sem):
        if kind == 'x':
            rows = pl.ds(XSPLIT[g], XSPLIT[g + 1] - XSPLIT[g])
            return pltpu.make_async_copy(x_hbm.at[rows], x_v.at[rows], sem)
        if kind == 'wq':
            return pltpu.make_async_copy(wq_hbm.at[:, pl.ds(g * GW, GW)], wq_v.at[g], sem)
        if kind == 'wq0':
            cols = pl.ds(g * (GW // 2), GW // 2)
            return pltpu.make_async_copy(wq_hbm.at[:, cols], wq_v.at[0, :, cols], sem)
        if kind == 'k':
            return pltpu.make_async_copy(k_hbm.at[:, pl.ds(g * G, G)], k_v.at[g], sem)
        if kind == 'v':
            return pltpu.make_async_copy(v_hbm.at[:, pl.ds(g * G, G)], v_v.at[g], sem)
        assert kind == 'wo'
        return pltpu.make_async_copy(wot_hbm.at[:, pl.ds(g * GW, GW)], wot_v.at[g], sem)

    def reg_copies(g, first=False):
        s = sems.at[S_REG + g]
        cs = [cp('k', g, s), cp('v', g, s), cp('wq', g + 2, s)]
        if not first:
            cs.append(cp('wo', g - 1, s))
        return cs

    pro = [[cp('x', 0, sems.at[0]), cp('wq0', 0, sems.at[0])], [cp('wq0', 1, sems.at[1])]]
    pro += [[cp('x', i, sems.at[i + 1])] for i in range(1, NX)]
    pro.append([cp('wq', 1, sems.at[S_WQ1])])
    ts = sems.at[S_TAIL]
    tail = [cp('wo', NG - 3, ts), cp('k', NG - 2, ts), cp('v', NG - 2, ts),
            cp('k', NG - 1, ts), cp('v', NG - 1, ts), cp('wo', NG - 2, ts), cp('wo', NG - 1, ts)]
    for cs in pro:
        for c in cs:
            c.start()
    for g in range(NG - 2):
        for c in reg_copies(g, g == 0):
            c.start()
    for c in tail:
        c.start()
    zs_ref[0] = 0
    acc_ref[...] = jnp.zeros_like(acc_ref)

    scale = DH ** -0.5 * LOG2E

    def task_a(g, slot, r0=0, r1=R, c0=0, c1=GW):
        q = jnp.dot(x_v[r0:r1, :], wq_v[g, :, c0:c1], preferred_element_type=jnp.float32)
        q_ref[slot, r0:r1, c0:c1] = (q * scale).astype(jnp.bfloat16)

    def task_b(g, qslot, oslot):
        pairs = [(b, j) for b in range(B) for j in range(G)]
        n = len(pairs)
        es = {}
        for st in range(0, n + LAG * W, W):
            for i in range(st, min(st + W, n)):
                b, j = pairs[i]
                qb = q_ref[qslot, b * SQ:(b + 1) * SQ, j * DH:(j + 1) * DH]
                s = jax.lax.dot_general(qb, k_v[g, b, j], NT, preferred_element_type=jnp.float32)
                m = jnp.max(s, axis=-1, keepdims=True)
                e = jnp.exp2(s - m)
                l = jnp.sum(e, axis=-1, keepdims=True)
                es[i] = (e.astype(jnp.bfloat16), pl.reciprocal(l, approx=True))
            for i in range(st - LAG * W, st - LAG * W + W):
                if 0 <= i < n:
                    b, j = pairs[i]
                    e, r = es.pop(i)
                    o = jnp.dot(e, v_v[g, b, j], preferred_element_type=jnp.float32)
                    oh_ref[oslot, b * SQ:(b + 1) * SQ, j * DH:(j + 1) * DH] = (o * r).astype(jnp.bfloat16)

    def proj_t(g, oslot, rows):
        return jax.lax.dot_general(wot_v[g], oh_ref[oslot, rows, 0:GW], NT,
                                   preferred_element_type=jnp.float32)

    def task_c(g, oslot):
        acc_ref[...] += proj_t(g, oslot, slice(0, R))

    for c in pro[0]:
        c.wait()
    task_a(0, 0, XSPLIT[0], XSPLIT[1], 0, GW // 2)
    for c in pro[1]:
        c.wait()
    task_a(0, 0, XSPLIT[0], XSPLIT[1], GW // 2, GW)
    for i in range(1, NX):
        for c in pro[i + 1]:
            c.wait()
        task_a(0, 0, XSPLIT[i], XSPLIT[i + 1])
    for c in pro[NX + 1]:
        c.wait()
    task_a(1, 1)
    for c in reg_copies(0, True):
        c.wait()
    task_b(0, 0, 0)
    task_a(2, 0)

    def loop_body(g, carry):
        for c in reg_copies(g):
            c.wait()
        task_c(g - 1, 0)
        task_b(g, g % 2, 0)
        task_a(g + 2, g % 2)
        return carry

    jax.lax.fori_loop(1, NG - 2, loop_body, 0)

    for c in tail:
        c.wait()
    g = NG - 2
    task_c(g - 1, 0)
    task_b(g, g % 2, 1)
    task_b(g + 1, (g + 1) % 2, 0)
    oslot = 2 + zs_ref[0]
    ntl = R // 128
    res = {}
    ocs = []

    def epi(t):
        oh_ref[oslot, t * 128:(t + 1) * 128, :] = res.pop(t).T.astype(jnp.bfloat16)
        oc = pltpu.make_async_copy(oh_ref.at[2, t * 128:(t + 1) * 128],
                                   o_hbm.at[t * 128:(t + 1) * 128], osem)
        oc.start()
        ocs.append(oc)

    for t in range(ntl):
        rows = slice(t * 128, (t + 1) * 128)
        pa = acc_ref[:, rows] + proj_t(g, 1, rows)
        if t == ntl - 1:
            epi(t - 1)
        res[t] = pa + proj_t(g + 1, 0, rows)
        if t >= 1 and (t - 1) in res:
            epi(t - 1)
    epi(ntl - 1)
    for oc in ocs:
        oc.wait()


@jax.jit
def pallas_standalone__mha_block_cached__near_ridge_kernel(
    x: jax.Array,
    k_cache: jax.Array,
    v_cache: jax.Array,
    wq: jax.Array,
    wo: jax.Array,
):
    bf16 = jnp.bfloat16
    out = pl.pallas_call(
        _body,
        in_specs=[pl.BlockSpec(memory_space=pl.ANY)] * 5,
        out_specs=pl.BlockSpec(memory_space=pl.ANY),
        out_shape=jax.ShapeDtypeStruct((R, D), bf16),
        scratch_shapes=[
            pltpu.VMEM((R, D), bf16),
            pltpu.VMEM((NG, B, G, SK, DH), bf16),
            pltpu.VMEM((NG, B, G, SK, DH), bf16),
            pltpu.VMEM((NG, D, GW), bf16),
            pltpu.VMEM((NG, D, GW), bf16),
            pltpu.VMEM((D, R), jnp.float32),
            pltpu.VMEM((2, R, GW), bf16),
            pltpu.VMEM((3, R, D), bf16),
            pltpu.SMEM((1,), jnp.int32),
            pltpu.SemaphoreType.DMA((NS,)),
            pltpu.SemaphoreType.DMA(()),
        ],
        compiler_params=pltpu.CompilerParams(vmem_limit_bytes=110 * 1024 * 1024),
    )(x.reshape(R, D), k_cache, v_cache, wq, wo.T)
    return out.reshape(B, SQ, D)
```

```python
import jax
import jax.numpy as jnp
import jax.experimental.pallas as pl
import jax.experimental.pallas.tpu as pltpu

B, SQ, D, H, SK, DH = 16, 64, 576, 32, 64, 128
R = B * SQ
G = 4
NG = H // G
GW = G * DH
LAG = 4
W = 4
XS = (0, 128, 384, 1024)
LOG2E = 1.4426950408889634
NT = (((1,), (1,)), ((), ()))

S_REG = 5
S_TAIL = S_REG + (NG - 2)
NS = S_TAIL + 1


def _body(x_hbm, k_hbm, v_hbm, wq_hbm, wot_hbm, o_hbm,
          x_v, k_v, v_v, wq_v, wot_v, acc_ref, q_ref, oh_ref, zs_ref, sems, osem):
    def cp(kind, g, sem):
        if kind == 'x':
            rows = pl.ds(XS[g], XS[g + 1] - XS[g])
            return pltpu.make_async_copy(x_hbm.at[rows], x_v.at[rows], sem)
        if kind == 'wq':
            return pltpu.make_async_copy(wq_hbm.at[:, pl.ds(g * GW, GW)], wq_v.at[g], sem)
        if kind == 'wq0':
            cols = pl.ds(g * (GW // 2), GW // 2)
            return pltpu.make_async_copy(wq_hbm.at[:, cols], wq_v.at[0, :, cols], sem)
        if kind == 'k':
            return pltpu.make_async_copy(k_hbm.at[:, pl.ds(g * G, G)], k_v.at[g], sem)
        if kind == 'v':
            return pltpu.make_async_copy(v_hbm.at[:, pl.ds(g * G, G)], v_v.at[g], sem)
        assert kind == 'wo'
        return pltpu.make_async_copy(wot_hbm.at[:, pl.ds(g * GW, GW)], wot_v.at[g], sem)

    def reg_copies(g):
        s = sems.at[S_REG + g]
        return [cp('k', g, s), cp('v', g, s), cp('wq', g + 2, s), cp('wo', g, s)]

    pro = [[cp('x', 0, sems.at[0]), cp('wq0', 0, sems.at[0])],
           [cp('wq0', 1, sems.at[1])],
           [cp('x', 1, sems.at[2])],
           [cp('wq', 1, sems.at[3])],
           [cp('x', 2, sems.at[4])]]
    ts = sems.at[S_TAIL]
    tail = [cp('k', NG - 2, ts), cp('v', NG - 2, ts), cp('k', NG - 1, ts), cp('v', NG - 1, ts),
            cp('wo', NG - 2, ts), cp('wo', NG - 1, ts)]
    for cs in pro:
        for c in cs:
            c.start()
    for g in range(NG - 2):
        for c in reg_copies(g):
            c.start()
    for c in tail:
        c.start()
    zs_ref[0] = 0
    acc_ref[...] = jnp.zeros_like(acc_ref)

    scale = DH ** -0.5 * LOG2E

    def task_a(g, slot, r0=0, r1=R, c0=0, c1=GW):
        q = jnp.dot(x_v[r0:r1, :], wq_v[g, :, c0:c1], preferred_element_type=jnp.float32)
        q_ref[slot, r0:r1, c0:c1] = (q * scale).astype(jnp.bfloat16)

    def task_b(gs):
        pairs = [(g, qs, os_, b, j) for (g, qs, os_) in gs for b in range(B) for j in range(G)]
        n = len(pairs)
        es = {}
        for st in range(0, n + LAG * W, W):
            for i in range(st, min(st + W, n)):
                g, qslot, oslot, b, j = pairs[i]
                qb = q_ref[qslot, b * SQ:(b + 1) * SQ, j * DH:(j + 1) * DH]
                s = jax.lax.dot_general(qb, k_v[g, b, j], NT, preferred_element_type=jnp.float32)
                m = jnp.max(s, axis=-1, keepdims=True)
                e = jnp.exp2(s - m)
                l = jnp.sum(e, axis=-1, keepdims=True)
                r = pl.reciprocal(l, approx=True)
                r = r * (2.0 - l * r)
                es[i] = (e.astype(jnp.bfloat16), r)
            for i in range(st - LAG * W, st - LAG * W + W):
                if 0 <= i < n:
                    g, qslot, oslot, b, j = pairs[i]
                    e, r = es.pop(i)
                    o = jnp.dot(e, v_v[g, b, j], preferred_element_type=jnp.float32)
                    oh_ref[oslot, b * SQ:(b + 1) * SQ, j * DH:(j + 1) * DH] = (o * r).astype(jnp.bfloat16)

    def proj_t(g, oslot, rows):
        return jax.lax.dot_general(wot_v[g], oh_ref[oslot, rows, 0:GW], NT,
                                   preferred_element_type=jnp.float32)

    for c in pro[0]:
        c.wait()
    task_a(0, 0, XS[0], XS[1], 0, GW // 2)
    for c in pro[1]:
        c.wait()
    task_a(0, 0, XS[0], XS[1], GW // 2, GW)
    for c in pro[2]:
        c.wait()
    task_a(0, 0, XS[1], XS[2])
    for c in pro[3]:
        c.wait()
    task_a(1, 1, XS[0], XS[2])
    for c in pro[4]:
        c.wait()
    task_a(0, 0, XS[2], XS[3])
    task_a(1, 1, XS[2], XS[3])

    def loop_body(g, carry):
        for c in reg_copies(g):
            c.wait()
        task_b([(g, g % 2, 0)])
        task_a(g + 2, g % 2)
        acc_ref[...] += proj_t(g, 0, slice(0, R))
        return carry

    jax.lax.fori_loop(0, NG - 2, loop_body, 0)

    for c in tail:
        c.wait()
    g = NG - 2
    task_b([(g, g % 2, 0), (g + 1, (g + 1) % 2, 1)])
    oslot = 2 + zs_ref[0]
    ntl = R // 128
    res = {}
    ocs = []

    def epi(t):
        rows = slice(t * 128, (t + 1) * 128)
        oh_ref[oslot, rows, :] = res.pop(t).T.astype(jnp.bfloat16)
        oc = pltpu.make_async_copy(oh_ref.at[oslot, rows], o_hbm.at[rows], osem)
        oc.start()
        ocs.append(oc)

    for t in range(ntl):
        rows = slice(t * 128, (t + 1) * 128)
        pa = acc_ref[:, rows] + proj_t(g, 0, rows)
        if t == ntl - 1:
            epi(t - 1)
        res[t] = pa + proj_t(g + 1, 1, rows)
        if t >= 1 and (t - 1) in res:
            epi(t - 1)
    epi(ntl - 1)
    for oc in ocs:
        oc.wait()


@jax.jit
def pallas_standalone__mha_block_cached__near_ridge_kernel(
    x: jax.Array,
    k_cache: jax.Array,
    v_cache: jax.Array,
    wq: jax.Array,
    wo: jax.Array,
):
    bf16 = jnp.bfloat16
    out = pl.pallas_call(
        _body,
        in_specs=[pl.BlockSpec(memory_space=pl.ANY)] * 5,
        out_specs=pl.BlockSpec(memory_space=pl.ANY),
        out_shape=jax.ShapeDtypeStruct((R, D), bf16),
        scratch_shapes=[
            pltpu.VMEM((R, D), bf16),
            pltpu.VMEM((NG, B, G, SK, DH), bf16),
            pltpu.VMEM((NG, B, G, SK, DH), bf16),
            pltpu.VMEM((NG, D, GW), bf16),
            pltpu.VMEM((NG, D, GW), bf16),
            pltpu.VMEM((D, R), jnp.float32),
            pltpu.VMEM((2, R, GW), bf16),
            pltpu.VMEM((3, R, D), bf16),
            pltpu.SMEM((1,), jnp.int32),
            pltpu.SemaphoreType.DMA((NS,)),
            pltpu.SemaphoreType.DMA(()),
        ],
        compiler_params=pltpu.CompilerParams(vmem_limit_bytes=110 * 1024 * 1024),
    )(x.reshape(R, D), k_cache, v_cache, wq, wo.T)
    return out.reshape(B, SQ, D)
```

```python
import jax
import jax.numpy as jnp
import jax.experimental.pallas as pl
import jax.experimental.pallas.tpu as pltpu

B, SQ, D, H, SK, DH = 16, 64, 576, 32, 64, 128
R = B * SQ
G = 4
NG = H // G
GW = G * DH
LAG = 4
W = 4
XS = (0, 128, 384, 1024)
LAG_T = 3
LOG2E = 1.4426950408889634
NT = (((1,), (1,)), ((), ()))
TN = (((0,), (0,)), ((), ()))

S_REG = 5
S_TAIL = S_REG + (NG - 2)
NS = S_TAIL + 1


def _body(x_hbm, k_hbm, v_hbm, wq_hbm, wot_hbm, o_hbm,
          x_v, k_v, v_v, wq_v, wot_v, acc_ref, q_ref, oh_ref, zs_ref, sems, osem):
    def cp(kind, g, sem):
        if kind == 'x':
            rows = pl.ds(XS[g], XS[g + 1] - XS[g])
            return pltpu.make_async_copy(x_hbm.at[rows], x_v.at[rows], sem)
        if kind == 'wq':
            return pltpu.make_async_copy(wq_hbm.at[:, pl.ds(g * GW, GW)], wq_v.at[g], sem)
        if kind == 'wq0':
            cols = pl.ds(g * (GW // 2), GW // 2)
            return pltpu.make_async_copy(wq_hbm.at[:, cols], wq_v.at[0, :, cols], sem)
        if kind == 'k':
            return pltpu.make_async_copy(k_hbm.at[:, pl.ds(g * G, G)], k_v.at[g], sem)
        if kind == 'v':
            return pltpu.make_async_copy(v_hbm.at[:, pl.ds(g * G, G)], v_v.at[g], sem)
        assert kind == 'wo'
        return pltpu.make_async_copy(wot_hbm.at[:, pl.ds(g * GW, GW)], wot_v.at[g], sem)

    def reg_copies(g):
        s = sems.at[S_REG + g]
        return [cp('k', g, s), cp('v', g, s), cp('wq', g + 2, s), cp('wo', g, s)]

    pro = [[cp('x', 0, sems.at[0]), cp('wq0', 0, sems.at[0])],
           [cp('wq0', 1, sems.at[1])],
           [cp('x', 1, sems.at[2])],
           [cp('wq', 1, sems.at[3])],
           [cp('x', 2, sems.at[4])]]
    ts = sems.at[S_TAIL]
    tail = [cp('k', NG - 2, ts), cp('v', NG - 2, ts), cp('k', NG - 1, ts), cp('v', NG - 1, ts),
            cp('wo', NG - 2, ts), cp('wo', NG - 1, ts)]
    for cs in pro:
        for c in cs:
            c.start()
    for g in range(NG - 2):
        for c in reg_copies(g):
            c.start()
    for c in tail:
        c.start()
    zs_ref[0] = 0
    acc_ref[...] = jnp.zeros_like(acc_ref)

    scale = DH ** -0.5 * LOG2E

    def task_a(g, slot, r0=0, r1=R, c0=0, c1=GW):
        q = jnp.dot(x_v[r0:r1, :], wq_v[g, :, c0:c1], preferred_element_type=jnp.float32)
        q_ref[slot, r0:r1, c0:c1] = (q * scale).astype(jnp.bfloat16)

    def rcp(l):
        r = pl.reciprocal(l, approx=True)
        return r * (2.0 - l * r)

    def task_b(g, qslot, oslot):
        pairs = [(b, j) for b in range(B) for j in range(G)]
        n = len(pairs)
        es = {}
        for st in range(0, n + LAG * W, W):
            for i in range(st, min(st + W, n)):
                b, j = pairs[i]
                qb = q_ref[qslot, b * SQ:(b + 1) * SQ, j * DH:(j + 1) * DH]
                s = jax.lax.dot_general(qb, k_v[g, b, j], NT, preferred_element_type=jnp.float32)
                m = jnp.max(s, axis=-1, keepdims=True)
                e = jnp.exp2(s - m)
                l = jnp.sum(e, axis=-1, keepdims=True)
                es[i] = (e.astype(jnp.bfloat16), rcp(l))
            for i in range(st - LAG * W, st - LAG * W + W):
                if 0 <= i < n:
                    b, j = pairs[i]
                    e, r = es.pop(i)
                    o = jnp.dot(e, v_v[g, b, j], preferred_element_type=jnp.float32)
                    oh_ref[oslot, b * SQ:(b + 1) * SQ, j * DH:(j + 1) * DH] = (o * r).astype(jnp.bfloat16)

    def task_bt(gs):
        units = [(g, qs, os_, bp, j) for (g, qs, os_) in gs for bp in range(B // 2) for j in range(G)]
        n = len(units)
        ps = {}
        lo = jax.lax.broadcasted_iota(jnp.int32, (SK, 2 * SQ), 1) < SQ
        for st in range(0, n + LAG_T * W, W):
            for i in range(st, min(st + W, n)):
                g, qslot, oslot, bp, j = units[i]
                q2 = q_ref[qslot, bp * 128:(bp + 1) * 128, j * DH:(j + 1) * DH]
                k2 = jnp.concatenate([k_v[g, 2 * bp, j], k_v[g, 2 * bp + 1, j]], axis=0)
                s2 = jax.lax.dot_general(k2, q2, NT, preferred_element_type=jnp.float32)
                st_ = jnp.where(lo, s2[0:SK], s2[SK:2 * SK])
                m = jnp.max(st_, axis=0, keepdims=True)
                e = jnp.exp2(st_ - m)
                p = e * rcp(jnp.sum(e, axis=0, keepdims=True))
                ps[i] = jnp.concatenate([jnp.where(lo, p, 0.0), jnp.where(lo, 0.0, p)],
                                        axis=0).astype(jnp.bfloat16)
            for i in range(st - LAG_T * W, st - LAG_T * W + W):
                if 0 <= i < n:
                    g, qslot, oslot, bp, j = units[i]
                    v2 = jnp.concatenate([v_v[g, 2 * bp, j], v_v[g, 2 * bp + 1, j]], axis=0)
                    o = jax.lax.dot_general(ps.pop(i), v2, TN, preferred_element_type=jnp.float32)
                    oh_ref[oslot, bp * 128:(bp + 1) * 128, j * DH:(j + 1) * DH] = o.astype(jnp.bfloat16)

    def proj_t(g, oslot, rows):
        return jax.lax.dot_general(wot_v[g], oh_ref[oslot, rows, 0:GW], NT,
                                   preferred_element_type=jnp.float32)

    for c in pro[0]:
        c.wait()
    task_a(0, 0, XS[0], XS[1], 0, GW // 2)
    for c in pro[1]:
        c.wait()
    task_a(0, 0, XS[0], XS[1], GW // 2, GW)
    for c in pro[2]:
        c.wait()
    task_a(0, 0, XS[1], XS[2])
    for c in pro[3]:
        c.wait()
    task_a(1, 1, XS[0], XS[2])
    for c in pro[4]:
        c.wait()
    task_a(0, 0, XS[2], XS[3])
    task_a(1, 1, XS[2], XS[3])

    def loop_body(g, carry):
        for c in reg_copies(g):
            c.wait()
        task_b(g, g % 2, 0)
        task_a(g + 2, g % 2)
        acc_ref[...] += proj_t(g, 0, slice(0, R))
        return carry

    jax.lax.fori_loop(0, NG - 2, loop_body, 0)

    for c in tail:
        c.wait()
    g = NG - 2
    task_bt([(g, g % 2, 0), (g + 1, (g + 1) % 2, 1)])
    oslot = 2 + zs_ref[0]
    ntl = R // 128
    res = {}
    ocs = []

    def write_out(t, val):
        rows = slice(t * 128, (t + 1) * 128)
        oh_ref[oslot, rows, :] = val.astype(jnp.bfloat16)
        oc = pltpu.make_async_copy(oh_ref.at[oslot, rows], o_hbm.at[rows], osem)
        oc.start()
        ocs.append(oc)

    last = slice((ntl - 1) * 128, ntl * 128)
    acc_last = acc_ref[:, last].T
    for t in range(ntl - 1):
        rows = slice(t * 128, (t + 1) * 128)
        res[t] = acc_ref[:, rows] + proj_t(g, 0, rows) + proj_t(g + 1, 1, rows)
        if t >= 1:
            write_out(t - 1, res.pop(t - 1).T)
    pa = acc_last + jax.lax.dot_general(oh_ref[0, last, 0:GW], wot_v[g], NT,
                                        preferred_element_type=jnp.float32)
    write_out(ntl - 2, res.pop(ntl - 2).T)
    write_out(ntl - 1, pa + jax.lax.dot_general(oh_ref[1, last, 0:GW], wot_v[g + 1], NT,
                                                preferred_element_type=jnp.float32))
    for oc in ocs:
        oc.wait()


@jax.jit
def pallas_standalone__mha_block_cached__near_ridge_kernel(
    x: jax.Array,
    k_cache: jax.Array,
    v_cache: jax.Array,
    wq: jax.Array,
    wo: jax.Array,
):
    bf16 = jnp.bfloat16
    out = pl.pallas_call(
        _body,
        in_specs=[pl.BlockSpec(memory_space=pl.ANY)] * 5,
        out_specs=pl.BlockSpec(memory_space=pl.ANY),
        out_shape=jax.ShapeDtypeStruct((R, D), bf16),
        scratch_shapes=[
            pltpu.VMEM((R, D), bf16),
            pltpu.VMEM((NG, B, G, SK, DH), bf16),
            pltpu.VMEM((NG, B, G, SK, DH), bf16),
            pltpu.VMEM((NG, D, GW), bf16),
            pltpu.VMEM((NG, D, GW), bf16),
            pltpu.VMEM((D, R), jnp.float32),
            pltpu.VMEM((2, R, GW), bf16),
            pltpu.VMEM((3, R, D), bf16),
            pltpu.SMEM((1,), jnp.int32),
            pltpu.SemaphoreType.DMA((NS,)),
            pltpu.SemaphoreType.DMA(()),
        ],
        compiler_params=pltpu.CompilerParams(vmem_limit_bytes=110 * 1024 * 1024),
    )(x.reshape(R, D), k_cache, v_cache, wq, wo.T)
    return out.reshape(B, SQ, D)
```

```python
import jax
import jax.numpy as jnp
import jax.experimental.pallas as pl
import jax.experimental.pallas.tpu as pltpu

B, SQ, D, H, SK, DH = 16, 64, 576, 32, 64, 128
R = B * SQ
G = 4
NG = H // G
GW = G * DH
LAG = 4
W = 4
XS = (0, 128, 384, 1024)
LAG_T = 3
LOG2E = 1.4426950408889634
NT = (((1,), (1,)), ((), ()))
TN = (((0,), (0,)), ((), ()))


def _body(x_hbm, k_hbm, v_hbm, wq_hbm, wot_hbm, o_hbm,
          x_v, k_v, v_v, wq_v, wot_v, acc_ref, q_ref, oh_ref, zs_ref, sems):
    def cp(kind, g, sem):
        if kind == 'x':
            rows = pl.ds(XS[g], XS[g + 1] - XS[g])
            return pltpu.make_async_copy(x_hbm.at[rows], x_v.at[rows], sem)
        if kind == 'wq':
            return pltpu.make_async_copy(wq_hbm.at[:, pl.ds(g * GW, GW)], wq_v.at[g], sem)
        if kind == 'wq0':
            cols = pl.ds(g * (GW // 2), GW // 2)
            return pltpu.make_async_copy(wq_hbm.at[:, cols], wq_v.at[0, :, cols], sem)
        if kind == 'k':
            return pltpu.make_async_copy(k_hbm.at[:, pl.ds(g * G, G)], k_v.at[g], sem)
        if kind == 'v':
            return pltpu.make_async_copy(v_hbm.at[:, pl.ds(g * G, G)], v_v.at[g], sem)
        assert kind == 'wo'
        return pltpu.make_async_copy(wot_hbm.at[:, pl.ds(g * GW, GW)], wot_v.at[g], sem)

    def reg_copies(g):
        s = sems.at[(g + 5) % 6 if isinstance(g, int) else jnp.where(g == 0, 5, g - 1)]
        return [cp('k', g, s), cp('v', g, s), cp('wq', g + 2, s), cp('wo', g, s)]

    def start(cs):
        for c in cs:
            c.start()

    def wait(cs):
        for c in cs:
            c.wait()

    pro = [[cp('x', 0, sems.at[0]), cp('wq0', 0, sems.at[0])],
           [cp('wq0', 1, sems.at[1])],
           [cp('x', 1, sems.at[2])],
           [cp('wq', 1, sems.at[3])],
           [cp('x', 2, sems.at[4])]]
    ts = sems.at[6]
    tail = [cp('k', NG - 2, ts), cp('v', NG - 2, ts), cp('k', NG - 1, ts), cp('v', NG - 1, ts),
            cp('wo', NG - 2, ts), cp('wo', NG - 1, ts)]
    for cs in pro:
        start(cs)
    start(reg_copies(0))
    zs_ref[0] = 0
    acc_ref[...] = jnp.zeros_like(acc_ref)

    scale = DH ** -0.5 * LOG2E

    def task_a(g, slot, r0=0, r1=R, c0=0, c1=GW):
        q = jnp.dot(x_v[r0:r1, :], wq_v[g, :, c0:c1], preferred_element_type=jnp.float32)
        q_ref[slot, r0:r1, c0:c1] = (q * scale).astype(jnp.bfloat16)

    def rcp(l):
        r = pl.reciprocal(l, approx=True)
        return r * (2.0 - l * r)

    def task_b(g, qslot, oslot):
        pairs = [(b, j) for b in range(B) for j in range(G)]
        n = len(pairs)
        es = {}
        for st in range(0, n + LAG * W, W):
            for i in range(st, min(st + W, n)):
                b, j = pairs[i]
                qb = q_ref[qslot, b * SQ:(b + 1) * SQ, j * DH:(j + 1) * DH]
                s = jax.lax.dot_general(qb, k_v[g, b, j], NT, preferred_element_type=jnp.float32)
                m = jnp.max(s, axis=-1, keepdims=True)
                e = jnp.exp2(s - m)
                l = jnp.sum(e, axis=-1, keepdims=True)
                es[i] = (e.astype(jnp.bfloat16), rcp(l))
            for i in range(st - LAG * W, st - LAG * W + W):
                if 0 <= i < n:
                    b, j = pairs[i]
                    e, r = es.pop(i)
                    o = jnp.dot(e, v_v[g, b, j], preferred_element_type=jnp.float32)
                    oh_ref[oslot, b * SQ:(b + 1) * SQ, j * DH:(j + 1) * DH] = (o * r).astype(jnp.bfloat16)

    def task_bt(gs):
        units = [(g, qs, os_, bp, j) for (g, qs, os_) in gs for bp in range(B // 2) for j in range(G)]
        n = len(units)
        ps = {}
        lo = jax.lax.broadcasted_iota(jnp.int32, (SK, 2 * SQ), 1) < SQ
        for st in range(0, n + LAG_T * W, W):
            for i in range(st, min(st + W, n)):
                g, qslot, oslot, bp, j = units[i]
                q2 = q_ref[qslot, bp * 128:(bp + 1) * 128, j * DH:(j + 1) * DH]
                k2 = jnp.concatenate([k_v[g, 2 * bp, j], k_v[g, 2 * bp + 1, j]], axis=0)
                s2 = jax.lax.dot_general(k2, q2, NT, preferred_element_type=jnp.float32)
                st_ = jnp.where(lo, s2[0:SK], s2[SK:2 * SK])
                m = jnp.max(st_, axis=0, keepdims=True)
                e = jnp.exp2(st_ - m)
                p = e * rcp(jnp.sum(e, axis=0, keepdims=True))
                ps[i] = jnp.concatenate([jnp.where(lo, p, 0.0), jnp.where(lo, 0.0, p)],
                                        axis=0).astype(jnp.bfloat16)
            for i in range(st - LAG_T * W, st - LAG_T * W + W):
                if 0 <= i < n:
                    g, qslot, oslot, bp, j = units[i]
                    v2 = jnp.concatenate([v_v[g, 2 * bp, j], v_v[g, 2 * bp + 1, j]], axis=0)
                    o = jax.lax.dot_general(ps.pop(i), v2, TN, preferred_element_type=jnp.float32)
                    oh_ref[oslot, bp * 128:(bp + 1) * 128, j * DH:(j + 1) * DH] = o.astype(jnp.bfloat16)

    def proj_t(g, oslot, rows):
        return jax.lax.dot_general(wot_v[g], oh_ref[oslot, rows, 0:GW], NT,
                                   preferred_element_type=jnp.float32)

    wait(pro[0])
    task_a(0, 0, XS[0], XS[1], 0, GW // 2)
    wait(pro[1])
    task_a(0, 0, XS[0], XS[1], GW // 2, GW)
    wait(pro[2])
    task_a(0, 0, XS[1], XS[2])
    wait(pro[3])
    task_a(1, 1, XS[0], XS[2])
    wait(pro[4])
    task_a(0, 0, XS[2], XS[3])
    for g in range(1, NG - 2):
        start(reg_copies(g))
    start(tail)
    task_a(1, 1, XS[2], XS[3])

    def loop_body(g, carry):
        wait(reg_copies(g))
        slot = jnp.bitwise_and(g, 1)
        task_b(g, slot, 0)
        task_a(g + 2, slot)
        acc_ref[...] += proj_t(g, 0, slice(0, R))
        return carry

    jax.lax.fori_loop(0, NG - 2, loop_body, 0)

    wait(tail)
    g = NG - 2
    task_bt([(g, g % 2, 0), (g + 1, (g + 1) % 2, 1)])
    oslot = 2 + zs_ref[0]
    ntl = R // 128
    res = {}
    ocs = []

    def start_out(t):
        rows = slice(t * 128, (t + 1) * 128)
        oc = pltpu.make_async_copy(oh_ref.at[oslot, rows], o_hbm.at[rows], sems.at[0])
        oc.start()
        ocs.append(oc)

    def write_out(t, val):
        oh_ref[oslot, t * 128:(t + 1) * 128, :] = val.astype(jnp.bfloat16)
        start_out(t)

    DM = (D // 128) * 128
    last = slice((ntl - 1) * 128, ntl * 128)
    acc_last = acc_ref[0:DM, last].T
    for t in range(ntl - 1):
        rows = slice(t * 128, (t + 1) * 128)
        res[t] = acc_ref[:, rows] + proj_t(g, 0, rows) + proj_t(g + 1, 1, rows)
        if t >= 1:
            write_out(t - 1, res.pop(t - 1).T)
    rem = (acc_ref[DM:D, last]
           + jax.lax.dot_general(wot_v[g, DM:D, :], oh_ref[0, last, 0:GW], NT,
                                 preferred_element_type=jnp.float32)
           + jax.lax.dot_general(wot_v[g + 1, DM:D, :], oh_ref[1, last, 0:GW], NT,
                                 preferred_element_type=jnp.float32))
    pa = acc_last + jax.lax.dot_general(oh_ref[0, last, 0:GW], wot_v[g, 0:DM, :], NT,
                                        preferred_element_type=jnp.float32)
    write_out(ntl - 2, res.pop(ntl - 2).T)
    oh_ref[oslot, last, DM:D] = rem.T.astype(jnp.bfloat16)
    oh_ref[oslot, last, 0:DM] = (pa + jax.lax.dot_general(
        oh_ref[1, last, 0:GW], wot_v[g + 1, 0:DM, :], NT,
        preferred_element_type=jnp.float32)).astype(jnp.bfloat16)
    start_out(ntl - 1)
    for oc in ocs:
        oc.wait()


@jax.jit
def pallas_standalone__mha_block_cached__near_ridge_kernel(
    x: jax.Array,
    k_cache: jax.Array,
    v_cache: jax.Array,
    wq: jax.Array,
    wo: jax.Array,
):
    bf16 = jnp.bfloat16
    out = pl.pallas_call(
        _body,
        in_specs=[pl.BlockSpec(memory_space=pl.ANY)] * 5,
        out_specs=pl.BlockSpec(memory_space=pl.ANY),
        out_shape=jax.ShapeDtypeStruct((R, D), bf16),
        scratch_shapes=[
            pltpu.VMEM((R, D), bf16),
            pltpu.VMEM((NG, B, G, SK, DH), bf16),
            pltpu.VMEM((NG, B, G, SK, DH), bf16),
            pltpu.VMEM((NG, D, GW), bf16),
            pltpu.VMEM((NG, D, GW), bf16),
            pltpu.VMEM((D, R), jnp.float32),
            pltpu.VMEM((2, R, GW), bf16),
            pltpu.VMEM((3, R, D), bf16),
            pltpu.SMEM((1,), jnp.int32),
            pltpu.SemaphoreType.DMA((7,)),
        ],
        compiler_params=pltpu.CompilerParams(vmem_limit_bytes=110 * 1024 * 1024),
    )(x.reshape(R, D), k_cache, v_cache, wq, wo.T)
    return out.reshape(B, SQ, D)
```

```python
import jax
import jax.numpy as jnp
import jax.experimental.pallas as pl
import jax.experimental.pallas.tpu as pltpu

B, SQ, D, H, SK, DH = 16, 64, 576, 32, 64, 128
R = B * SQ
G = 4
NG = H // G
GW = G * DH
LAG = 4
W = 4
XS = (0, 128, 384, 1024)
LAG_T = 3
LOG2E = 1.4426950408889634
NT = (((1,), (1,)), ((), ()))
TN = (((0,), (0,)), ((), ()))


def _body(x_hbm, k_hbm, v_hbm, wq_hbm, wot_hbm, o_hbm,
          x_v, k_v, v_v, wq_v, wot_v, acc_ref, q_ref, oh_ref, zs_ref, sems):
    def cp(kind, g, sem):
        if kind == 'x':
            rows = pl.ds(XS[g], XS[g + 1] - XS[g])
            return pltpu.make_async_copy(x_hbm.at[rows], x_v.at[rows], sem)
        if kind == 'wq':
            return pltpu.make_async_copy(wq_hbm.at[:, pl.ds(g * GW, GW)], wq_v.at[g], sem)
        if kind == 'wq0':
            cols = pl.ds(g * (GW // 2), GW // 2)
            return pltpu.make_async_copy(wq_hbm.at[:, cols], wq_v.at[0, :, cols], sem)
        if kind == 'k':
            return pltpu.make_async_copy(k_hbm.at[:, pl.ds(g * G, G)], k_v.at[g], sem)
        if kind == 'v':
            return pltpu.make_async_copy(v_hbm.at[:, pl.ds(g * G, G)], v_v.at[g], sem)
        assert kind == 'wo'
        return pltpu.make_async_copy(wot_hbm.at[:, pl.ds(g * GW, GW)], wot_v.at[g], sem)

    def reg_copies(g):
        s = sems.at[(g + 5) % 6 if isinstance(g, int) else jnp.where(g == 0, 5, g - 1)]
        return [cp('k', g, s), cp('v', g, s), cp('wq', g + 2, s), cp('wo', g, s)]

    def start(cs):
        for c in cs:
            c.start()

    def wait(cs):
        for c in cs:
            c.wait()

    pro = [[cp('wq0', 0, sems.at[0]), cp('x', 0, sems.at[0])],
           [cp('x', 1, sems.at[1])],
           [cp('wq0', 1, sems.at[2])],
           [cp('wq', 1, sems.at[3])],
           [cp('x', 2, sems.at[4])]]
    ts = sems.at[6]
    tail = [cp('k', NG - 2, ts), cp('v', NG - 2, ts), cp('k', NG - 1, ts), cp('v', NG - 1, ts),
            cp('wo', NG - 2, ts), cp('wo', NG - 1, ts)]
    for cs in pro:
        start(cs)
    start(reg_copies(0))
    zs_ref[0] = 0
    acc_ref[...] = jnp.zeros_like(acc_ref)

    scale = DH ** -0.5 * LOG2E

    def task_a(g, slot, r0=0, r1=R, c0=0, c1=GW):
        q = jnp.dot(x_v[r0:r1, :], wq_v[g, :, c0:c1], preferred_element_type=jnp.float32)
        q_ref[slot, r0:r1, c0:c1] = (q * scale).astype(jnp.bfloat16)

    def rcp(l):
        r = pl.reciprocal(l, approx=True)
        return r * (2.0 - l * r)

    def task_b(g, qslot, oslot):
        pairs = [(b, j) for b in range(B) for j in range(G)]
        n = len(pairs)
        es = {}
        for st in range(0, n + LAG * W, W):
            for i in range(st, min(st + W, n)):
                b, j = pairs[i]
                qb = q_ref[qslot, b * SQ:(b + 1) * SQ, j * DH:(j + 1) * DH]
                s = jax.lax.dot_general(qb, k_v[g, b, j], NT, preferred_element_type=jnp.float32)
                m = jnp.max(s, axis=-1, keepdims=True)
                e = jnp.exp2(s - m)
                l = jnp.sum(e, axis=-1, keepdims=True)
                es[i] = (e.astype(jnp.bfloat16), rcp(l))
            for i in range(st - LAG * W, st - LAG * W + W):
                if 0 <= i < n:
                    b, j = pairs[i]
                    e, r = es.pop(i)
                    o = jnp.dot(e, v_v[g, b, j], preferred_element_type=jnp.float32)
                    oh_ref[oslot, b * SQ:(b + 1) * SQ, j * DH:(j + 1) * DH] = (o * r).astype(jnp.bfloat16)

    def task_bt(gs):
        units = [(g, qs, os_, bp, j) for (g, qs, os_) in gs for bp in range(B // 2) for j in range(G)]
        n = len(units)
        ps = {}
        lo = jax.lax.broadcasted_iota(jnp.int32, (SK, 2 * SQ), 1) < SQ
        for st in range(0, n + LAG_T * W, W):
            for i in range(st, min(st + W, n)):
                g, qslot, oslot, bp, j = units[i]
                q2 = q_ref[qslot, bp * 128:(bp + 1) * 128, j * DH:(j + 1) * DH]
                k2 = jnp.concatenate([k_v[g, 2 * bp, j], k_v[g, 2 * bp + 1, j]], axis=0)
                s2 = jax.lax.dot_general(k2, q2, NT, preferred_element_type=jnp.float32)
                st_ = jnp.where(lo, s2[0:SK], s2[SK:2 * SK])
                m = jnp.max(st_, axis=0, keepdims=True)
                e = jnp.exp2(st_ - m)
                p = e * rcp(jnp.sum(e, axis=0, keepdims=True))
                ps[i] = jnp.concatenate([jnp.where(lo, p, 0.0), jnp.where(lo, 0.0, p)],
                                        axis=0).astype(jnp.bfloat16)
            for i in range(st - LAG_T * W, st - LAG_T * W + W):
                if 0 <= i < n:
                    g, qslot, oslot, bp, j = units[i]
                    v2 = jnp.concatenate([v_v[g, 2 * bp, j], v_v[g, 2 * bp + 1, j]], axis=0)
                    o = jax.lax.dot_general(ps.pop(i), v2, TN, preferred_element_type=jnp.float32)
                    oh_ref[oslot, bp * 128:(bp + 1) * 128, j * DH:(j + 1) * DH] = o.astype(jnp.bfloat16)

    def proj_t(g, oslot, rows):
        return jax.lax.dot_general(wot_v[g], oh_ref[oslot, rows, 0:GW], NT,
                                   preferred_element_type=jnp.float32)

    hw = GW // 2
    wait(pro[0])
    task_a(0, 0, 0, 64, 0, hw)
    task_a(0, 0, 64, 128, 0, hw)
    wait(pro[1])
    task_a(0, 0, 128, 256, 0, hw)
    task_a(0, 0, 256, 384, 0, hw)
    wait(pro[2])
    task_a(0, 0, 0, 192, hw, GW)
    task_a(0, 0, 192, 384, hw, GW)
    wait(pro[3])
    task_a(1, 1, XS[0], XS[2])
    wait(pro[4])
    task_a(0, 0, XS[2], XS[3])
    for g in range(1, NG - 2):
        start(reg_copies(g))
    start(tail)
    task_a(1, 1, XS[2], XS[3])

    def loop_body(g, carry):
        wait(reg_copies(g))
        slot = jnp.bitwise_and(g, 1)
        task_b(g, slot, 0)
        task_a(g + 2, slot)
        acc_ref[...] += proj_t(g, 0, slice(0, R))
        return carry

    jax.lax.fori_loop(0, NG - 2, loop_body, 0)

    wait(tail)
    g = NG - 2
    task_bt([(g, g % 2, 0), (g + 1, (g + 1) % 2, 1)])
    oslot = 2 + zs_ref[0]
    ntl = R // 128
    res = {}
    ocs = []

    def start_out(t):
        rows = slice(t * 128, (t + 1) * 128)
        oc = pltpu.make_async_copy(oh_ref.at[oslot, rows], o_hbm.at[rows], sems.at[0])
        oc.start()
        ocs.append(oc)

    def write_out(t, val):
        oh_ref[oslot, t * 128:(t + 1) * 128, :] = val.astype(jnp.bfloat16)
        start_out(t)

    DM = (D // 128) * 128
    last = slice((ntl - 1) * 128, ntl * 128)
    acc_last = acc_ref[0:DM, last].T
    for t in range(ntl - 1):
        rows = slice(t * 128, (t + 1) * 128)
        res[t] = acc_ref[:, rows] + proj_t(g, 0, rows) + proj_t(g + 1, 1, rows)
        if t >= 1:
            write_out(t - 1, res.pop(t - 1).T)
    rem = (acc_ref[DM:D, last]
           + jax.lax.dot_general(wot_v[g, DM:D, :], oh_ref[0, last, 0:GW], NT,
                                 preferred_element_type=jnp.float32)
           + jax.lax.dot_general(wot_v[g + 1, DM:D, :], oh_ref[1, last, 0:GW], NT,
                                 preferred_element_type=jnp.float32))
    pa = acc_last + jax.lax.dot_general(oh_ref[0, last, 0:GW], wot_v[g, 0:DM, :], NT,
                                        preferred_element_type=jnp.float32)
    write_out(ntl - 2, res.pop(ntl - 2).T)
    oh_ref[oslot, last, DM:D] = rem.T.astype(jnp.bfloat16)
    oh_ref[oslot, last, 0:DM] = (pa + jax.lax.dot_general(
        oh_ref[1, last, 0:GW], wot_v[g + 1, 0:DM, :], NT,
        preferred_element_type=jnp.float32)).astype(jnp.bfloat16)
    start_out(ntl - 1)
    for oc in ocs:
        oc.wait()


@jax.jit
def pallas_standalone__mha_block_cached__near_ridge_kernel(
    x: jax.Array,
    k_cache: jax.Array,
    v_cache: jax.Array,
    wq: jax.Array,
    wo: jax.Array,
):
    bf16 = jnp.bfloat16
    out = pl.pallas_call(
        _body,
        in_specs=[pl.BlockSpec(memory_space=pl.ANY)] * 5,
        out_specs=pl.BlockSpec(memory_space=pl.ANY),
        out_shape=jax.ShapeDtypeStruct((R, D), bf16),
        scratch_shapes=[
            pltpu.VMEM((R, D), bf16),
            pltpu.VMEM((NG, B, G, SK, DH), bf16),
            pltpu.VMEM((NG, B, G, SK, DH), bf16),
            pltpu.VMEM((NG, D, GW), bf16),
            pltpu.VMEM((NG, D, GW), bf16),
            pltpu.VMEM((D, R), jnp.float32),
            pltpu.VMEM((2, R, GW), bf16),
            pltpu.VMEM((3, R, D), bf16),
            pltpu.SMEM((1,), jnp.int32),
            pltpu.SemaphoreType.DMA((7,)),
        ],
        compiler_params=pltpu.CompilerParams(vmem_limit_bytes=110 * 1024 * 1024),
    )(x.reshape(R, D), k_cache, v_cache, wq, wo.T)
    return out.reshape(B, SQ, D)
```
